```python
import os as _os
_os.environ.setdefault("JAX_PLATFORMS", "cpu")
import jax
import jax.numpy as jnp

def _softmax(x, axis=-1):
    return jax.nn.softmax(x, axis=axis)
def _gelu(x):
    return jax.nn.gelu(x, approximate=True)
def _silu(x):
    return jax.nn.silu(x)
def _sigmoid(x):
    return jax.nn.sigmoid(x)
def _layernorm(x, axis=-1, eps=1e-5):
    m = jnp.mean(x, axis=axis, keepdims=True)
    v = jnp.var(x, axis=axis, keepdims=True)
    return (x - m) / jnp.sqrt(v + eps)
def _scatter_add(tgt, idx, src, axis=0):
    return tgt.at[idx].add(src)
def _segment_sum(src, seg, n):
    return jax.ops.segment_sum(src, seg, n)
class _Rng:
    def __init__(self, key):
        self._k = key
    def _next(self):
        self._k, sub = jax.random.split(self._k)
        return sub
    def normal(self, shape):
        return jax.random.normal(self._next(), shape, dtype=jnp.bfloat16)
    def randint(self, lo, hi, shape):
        return jax.random.randint(self._next(), shape, lo, hi, dtype=jnp.int32)
    def uniform(self, shape, lo=0.0, hi=1.0):
        return jax.random.uniform(self._next(), shape, jnp.bfloat16, lo, hi)
    def permutation(self, n):
        return jax.random.permutation(self._next(), n)


kernel_name = 'parallel_sum__linear_kernel_hedgehog__dense_activation_gelu__prompt'

def setup_inputs():
    _rng = _Rng(jax.random.key(int.from_bytes(__import__("os").urandom(4), "little")))
    _w = (lambda a: (lambda t: t.astype(jnp.bfloat16) if jnp.issubdtype(t.dtype, jnp.floating) else t)(jnp.asarray(a)))
    def _A_setup():
        B, S, D, H = 1, 2048, 448, 16
        Dh = D // H
        return {
            "x": _w((lambda *s: _rng.normal(s) * 0.05)(B, S, D)),
            "wqkv": _w((lambda *s: _rng.normal(s) * 0.2)(D, 3 * D)),
            "w_phi": _w((lambda *s: _rng.normal(s) * 0.2)(H, Dh, Dh) * (Dh ** -0.5)),
            "wo": _w((lambda *s: _rng.normal(s) * 0.05)(D, D)),
        }
    _A_in = _A_setup()

    def _B_setup():
        B, S, D, F = 1, 2048, 448, 1792
        return {
            "x": _w((lambda *s: _rng.normal(s) * 0.05)(B, S, D)),
            "w1": _w((lambda *s: _rng.normal(s) * 0.2)(D, F) * (D ** -0.5)),
            "b1": _w((lambda *s: _rng.normal(s) * 0.2)(F) * 0.01),
            "w2": _w((lambda *s: _rng.normal(s) * 0.2)(F, D) * (F ** -0.5)),
            "b2": _w((lambda *s: _rng.normal(s) * 0.05)(D) * 0.01),
        }
    _B_in = _B_setup()

    return {
        "A_x": _A_in["x"],
        "A_wqkv": _A_in["wqkv"],
        "A_w_phi": _A_in["w_phi"],
        "A_wo": _A_in["wo"],
        "B_x": _B_in["x"],
        "B_w1": _B_in["w1"],
        "B_b1": _B_in["b1"],
        "B_w2": _B_in["w2"],
        "B_b2": _B_in["b2"],
    }

def reference(A_x, A_wqkv, A_w_phi, A_wo, B_x, B_w1, B_b1, B_w2, B_b2):
    def _A_ref(x, wqkv, w_phi, wo):
        B, S, D = x.shape
        H = 16; Dh = D // H
        qkv = (lambda x, *d: x.transpose(*d))((x @ wqkv).reshape(B, S, 3, H, Dh), 2, 0, 3, 1, 4)
        q, k, v = qkv[0], qkv[1], qkv[2]
        pq = jnp.einsum("bhsd,hdf->bhsf", q, w_phi)
        pk = jnp.einsum("bhsd,hdf->bhsf", k, w_phi)
        phi_q = jnp.concatenate([_softmax(pq, axis=-1), _softmax(-pq, axis=-1)], axis=-1)
        phi_k = jnp.concatenate([_softmax(pk, axis=-1), _softmax(-pk, axis=-1)], axis=-1)
        kv = jnp.einsum("bhsf,bhsd->bhfd", phi_k, v)
        z  = jnp.einsum("bhsf->bhf", phi_k)
        num = jnp.einsum("bhqf,bhfd->bhqd", phi_q, kv)
        den = jnp.einsum("bhqf,bhf->bhq", phi_q, z)[..., None] + 1e-6
        o = num / den
        return (lambda x, *d: x.transpose(*d))(o, 0, 2, 1, 3).reshape(B, S, D) @ wo

    def _B_ref(x, w1, b1, w2, b2):
        h = jnp.einsum("bsd,df->bsf", x, w1) + b1
        h = _gelu(h)
        return jnp.einsum("bsf,fd->bsd", h, w2) + b2

    x = A_x
    xn = _layernorm(x, axis=-1)
    return x + _A_ref(xn, A_wqkv, A_w_phi, A_wo) + _B_ref(xn, B_w1, B_b1, B_w2, B_b2)
```

```python
import functools
import jax
import jax.numpy as jnp
from jax import lax
import jax.experimental.pallas as pl
import jax.experimental.pallas.tpu as pltpu

H = 16
HP = 32
T = 256
F32 = jnp.float32
BF16 = jnp.bfloat16
NT = (((1,), (1,)), ((), ()))
TN = (((0,), (0,)), ((), ()))
NN = (((1,), (0,)), ((), ()))


def _dot(a, b, dims):
    return lax.dot_general(a, b, dims, preferred_element_type=F32)


def _dual_softmax(p, dh):
    t = p.shape[1]
    p = p.reshape(H, HP, t)
    row = lax.broadcasted_iota(jnp.int32, (1, HP, t), 1)
    nm = jnp.where(row < dh, 0.0, -jnp.inf).astype(F32)
    outs = []
    for a in (p + nm, nm - p):
        e = jnp.exp(a - jnp.max(a, axis=1, keepdims=True))
        s = jnp.sum(e, axis=1, keepdims=True)
        outs.append((e * (1.0 / s)).reshape(H * HP, t).astype(BF16))
    return outs


def _gelu(h):
    c = 0.7978845608028654
    u = h * (c + (c * 0.044715) * (h * h))
    hh = 0.5 * h
    return hh + hh * jnp.tanh(u)


def _kernel(x_hbm, wqkv_hbm, phi_ref, wo_hbm, w1_hbm, b1_ref, w2_hbm, b2_ref, o_hbm,
            x_v, xn_v, wqkv_v, wo_v, w1_v, w2_v, m_v, wt_v, wop_v, kv_v, kvb_v, ob_v,
            sem_x, sem_w, sem_o, *, S, D, FF):
    dh = D // H
    nt = S // T
    G = H * HP // 128

    def xcp(i):
        return pltpu.make_async_copy(x_hbm.at[pl.ds(i * T, T)], x_v.at[pl.ds(i * T, T)], sem_x.at[i])

    c_qkv = pltpu.make_async_copy(wqkv_hbm, wqkv_v, sem_w.at[0])
    c_w1 = pltpu.make_async_copy(w1_hbm, w1_v, sem_w.at[1])
    c_w2 = pltpu.make_async_copy(w2_hbm, w2_v, sem_w.at[2])
    c_wo = pltpu.make_async_copy(wo_hbm, wo_v, sem_w.at[3])
    c_qkv.start()
    for i in range(nt):
        xcp(i).start()
    c_wo.start()
    c_w1.start()
    c_w2.start()

    ri = lax.broadcasted_iota(jnp.int32, (D, H * HP), 0)
    ci = lax.broadcasted_iota(jnp.int32, (D, H * HP), 1)
    sel = ((ci % HP < dh) & ((ci // HP) * dh + ci % HP == ri)).astype(F32)
    m_v[pl.ds(0, 2 * D), :] = jnp.zeros((2 * D, H * HP), F32)
    m_v[pl.ds(2 * D, D), :] = sel
    for h in range(H):
        blk = phi_ref[h].astype(F32)
        m_v[h * dh:(h + 1) * dh, h * HP:h * HP + dh] = blk
        m_v[D + h * dh:D + (h + 1) * dh, h * HP:h * HP + dh] = blk
    kv_v[...] = jnp.zeros(kv_v.shape, F32)
    c_qkv.wait()

    def fold(j):
        for g in range(G):
            a = (j * D + g * 4 * dh) // 128 * 128
            b = min(a + 256, 3 * D)
            mg = m_v[a:b, g * 128:(g + 1) * 128].astype(BF16)
            r = lax.dot_general(mg, wqkv_v[:, a:b], (((0,), (1,)), ((), ())), preferred_element_type=F32)
            wt_v[(j * G + g) * 128:(j * G + g + 1) * 128, :] = r.astype(BF16)

    fold(1)
    fold(2)
    r2 = lax.broadcasted_iota(jnp.int32, (H * HP, T), 0)
    ones_row = (r2 % HP == dh).astype(F32)

    def phase1(i, c):
        st = pl.multiple_of(i * T, T)
        xcp(i).wait()
        x = x_v[pl.ds(st, T), :].astype(F32)
        mu = jnp.mean(x, axis=-1, keepdims=True)
        xc = x - mu
        var = jnp.mean(xc * xc, axis=-1, keepdims=True)
        xn = (xc * lax.rsqrt(var + 1e-5)).astype(BF16)
        xn_v[pl.ds(st, T), :] = xn
        pk = _dot(wt_v[H * HP:2 * H * HP, :], xn, NT)
        vt = (_dot(wt_v[2 * H * HP:, :], xn, NT) + ones_row).astype(BF16)
        kp, kn = _dual_softmax(pk, dh)
        for g in range(G):
            sl = slice(g * 128, (g + 1) * 128)
            kv_v[g, :, 0:128] += _dot(vt[sl], kp[sl], NT)
            kv_v[g, :, 128:256] += _dot(vt[sl], kn[sl], NT)
        return c

    lax.fori_loop(0, nt, phase1, 0)

    fold(0)
    rr = lax.broadcasted_iota(jnp.int32, (128, 256), 0)
    cc = lax.broadcasted_iota(jnp.int32, (128, 256), 1)
    diag = (rr // HP) == ((cc % 128) // HP)
    for g in range(G):
        kvb_v[g] = jnp.where(diag, kv_v[g], 0.0).astype(BF16)
    c_wo.wait()
    wop_v[...] = _dot(m_v[pl.ds(2 * D, D), :].astype(BF16), wo_v[...], TN).astype(BF16)
    c_w1.wait()
    c_w2.wait()

    def ocp(i, slot):
        return pltpu.make_async_copy(ob_v.at[slot], o_hbm.at[pl.ds(pl.multiple_of(i * T, T), T)], sem_o.at[slot])

    def phase2(i, c):
        st = pl.multiple_of(i * T, T)
        slot = i % 2
        xn = xn_v[pl.ds(st, T), :]
        pq = _dot(wt_v[0:H * HP, :], xn, NT)
        qp, qn = _dual_softmax(pq, dh)
        os_ = []
        for g in range(G):
            sl = slice(g * 128, (g + 1) * 128)
            num = _dot(kvb_v[g, :, 0:128], qp[sl], NN) + _dot(kvb_v[g, :, 128:256], qn[sl], NN)
            num = num.reshape(4, HP, T)
            den = num[:, dh:dh + 1, :] + 1e-6
            os_.append((num * (1.0 / den)).reshape(128, T).astype(BF16))
        ot = jnp.concatenate(os_, axis=0)
        hid = _gelu(_dot(xn, w1_v[...], NN) + b1_ref[...].astype(F32)).astype(BF16)
        acc = _dot(hid, w2_v[...], NN) + _dot(ot, wop_v[...], TN)
        acc = acc + b2_ref[...].astype(F32) + x_v[pl.ds(st, T), :].astype(F32)

        @pl.when(i >= 2)
        def _():
            ocp(i - 2, slot).wait()
        ob_v[slot] = acc.astype(BF16)
        ocp(i, slot).start()
        return c

    lax.fori_loop(0, nt, phase2, 0)
    ocp(nt - 2, nt % 2).wait()
    ocp(nt - 1, (nt - 1) % 2).wait()


@jax.jit
def pallas_parallel_sum__linear_kernel_hedgehog__dense_activation_gelu__prompt_kernel(
    A_x, A_wqkv, A_w_phi, A_wo, B_x, B_w1, B_b1, B_w2, B_b2,
):
    B, S, D = A_x.shape
    FF = B_w1.shape[1]
    x = A_x.reshape(S, D)
    any_ = pl.BlockSpec(memory_space=pl.ANY)
    vm = pl.BlockSpec(memory_space=pltpu.VMEM)
    out = pl.pallas_call(
        functools.partial(_kernel, S=S, D=D, FF=FF),
        in_specs=[any_, any_, vm, any_, any_, vm, any_, vm],
        out_specs=any_,
        out_shape=jax.ShapeDtypeStruct((S, D), A_x.dtype),
        scratch_shapes=[
            pltpu.VMEM((S, D), BF16), pltpu.VMEM((S, D), BF16),
            pltpu.VMEM((D, 3 * D), BF16), pltpu.VMEM((D, D), BF16),
            pltpu.VMEM((D, FF), BF16), pltpu.VMEM((FF, D), BF16),
            pltpu.VMEM((3 * D + 64, H * HP), F32), pltpu.VMEM((3 * H * HP, D), BF16),
            pltpu.VMEM((H * HP, D), BF16),
            pltpu.VMEM((4, 128, 256), F32), pltpu.VMEM((4, 128, 256), BF16),
            pltpu.VMEM((2, T, D), BF16),
            pltpu.SemaphoreType.DMA((S // T,)), pltpu.SemaphoreType.DMA((4,)),
            pltpu.SemaphoreType.DMA((2,)),
        ],
        compiler_params=pltpu.CompilerParams(vmem_limit_bytes=64 * 1024 * 1024),
    )(x, A_wqkv, A_w_phi, A_wo, B_w1, B_b1.reshape(1, FF), B_w2, B_b2.reshape(1, D))
    return out.reshape(B, S, D)
```

```python
import functools
import jax
import jax.numpy as jnp
from jax import lax
import jax.experimental.pallas as pl
import jax.experimental.pallas.tpu as pltpu

H = 16
HP = 32
T = 512
F32 = jnp.float32
BF16 = jnp.bfloat16
NT = (((1,), (1,)), ((), ()))
TN = (((0,), (0,)), ((), ()))
NN = (((1,), (0,)), ((), ()))


def _dot(a, b, dims):
    return lax.dot_general(a, b, dims, preferred_element_type=F32)


def _dual_softmax(p, dh):
    t = p.shape[1]
    p = p.reshape(H, HP, t)
    row = lax.broadcasted_iota(jnp.int32, (1, HP, t), 1)
    nm = jnp.where(row < dh, 0.0, -jnp.inf).astype(F32)
    outs = []
    for a in (p + nm, nm - p):
        e = jnp.exp(a - jnp.max(a, axis=1, keepdims=True))
        s = jnp.sum(e, axis=1, keepdims=True)
        outs.append((e * (1.0 / s)).reshape(H * HP, t).astype(BF16))
    return outs


def _gelu(h):
    c = 0.7978845608028654
    u = h * (c + (c * 0.044715) * (h * h))
    hh = 0.5 * h
    return hh + hh * jnp.tanh(u)


def _kernel(x_hbm, wqkv_hbm, phi_ref, wo_hbm, w1_hbm, b1_ref, w2_hbm, b2_ref, o_hbm,
            x_v, xn_v, wqkv_v, wo_v, w1_v, w2_v, m_v, wt_v, wop_v, w1t_v, b1_v, b2_v, kv_v, kvb_v, ob_v,
            sem_x, sem_w, sem_o, *, S, D, FF):
    dh = D // H
    nt = S // T
    G = H * HP // 128

    def xcp(i):
        return pltpu.make_async_copy(x_hbm.at[:, pl.ds(pl.multiple_of(i * T, T), T)], x_v.at[:, pl.ds(pl.multiple_of(i * T, T), T)], sem_x.at[i])

    c_qkv = pltpu.make_async_copy(wqkv_hbm, wqkv_v, sem_w.at[0])
    c_w1 = pltpu.make_async_copy(w1_hbm, w1_v, sem_w.at[1])
    c_w2 = pltpu.make_async_copy(w2_hbm, w2_v, sem_w.at[2])
    c_wo = pltpu.make_async_copy(wo_hbm, wo_v, sem_w.at[3])
    c_qkv.start()
    for i in range(nt):
        xcp(i).start()
    c_wo.start()
    c_w1.start()
    c_w2.start()

    ri = lax.broadcasted_iota(jnp.int32, (D, H * HP), 0)
    ci = lax.broadcasted_iota(jnp.int32, (D, H * HP), 1)
    sel = ((ci % HP < dh) & ((ci // HP) * dh + ci % HP == ri)).astype(F32)
    m_v[pl.ds(0, 2 * D), :] = jnp.zeros((2 * D, H * HP), F32)
    m_v[pl.ds(2 * D, D), :] = sel
    for h in range(H):
        blk = phi_ref[:, h, :].astype(F32)
        m_v[h * dh:(h + 1) * dh, h * HP:h * HP + dh] = blk
        m_v[D + h * dh:D + (h + 1) * dh, h * HP:h * HP + dh] = blk
    kv_v[...] = jnp.zeros(kv_v.shape, F32)
    c_qkv.wait()

    def fold(j):
        for g in range(G):
            a = (j * D + g * 4 * dh) // 128 * 128
            b = min(a + 256, 3 * D)
            mg = m_v[a:b, g * 128:(g + 1) * 128].astype(BF16)
            r = lax.dot_general(mg, wqkv_v[:, a:b], (((0,), (1,)), ((), ())), preferred_element_type=F32)
            wt_v[(j * G + g) * 128:(j * G + g + 1) * 128, :] = r.astype(BF16)

    fold(1)
    fold(2)
    r2 = lax.broadcasted_iota(jnp.int32, (H * HP, T), 0)
    ones_row = (r2 % HP == dh).astype(F32)

    def phase1(i, c):
        st = pl.multiple_of(i * T, T)
        xcp(i).wait()
        x = x_v[:, pl.ds(st, T)].astype(F32)
        mu = jnp.mean(x, axis=0, keepdims=True)
        xc = x - mu
        var = jnp.mean(xc * xc, axis=0, keepdims=True)
        xn = (xc * lax.rsqrt(var + 1e-5)).astype(BF16)
        xn_v[:, pl.ds(st, T)] = xn
        pk = _dot(wt_v[H * HP:2 * H * HP, :], xn, NN)
        vt = (_dot(wt_v[2 * H * HP:, :], xn, NN) + ones_row).astype(BF16)
        kp, kn = _dual_softmax(pk, dh)
        for g in range(G):
            sl = slice(g * 128, (g + 1) * 128)
            kv_v[g, :, 0:128] += _dot(vt[sl], kp[sl], NT)
            kv_v[g, :, 128:256] += _dot(vt[sl], kn[sl], NT)
        return c

    lax.fori_loop(0, nt, phase1, 0)

    fold(0)
    rr = lax.broadcasted_iota(jnp.int32, (128, 256), 0)
    cc = lax.broadcasted_iota(jnp.int32, (128, 256), 1)
    diag = (rr // HP) == ((cc % 128) // HP)
    for g in range(G):
        kvb_v[g] = jnp.where(diag, kv_v[g], 0.0).astype(BF16)
    c_wo.wait()
    wop_v[...] = _dot(wo_v[...], m_v[pl.ds(2 * D, D), :].astype(BF16), TN).astype(BF16)
    b1_v[...] = jnp.broadcast_to(b1_ref[...].astype(F32)[None, :], (128, FF)).T
    b2_v[...] = jnp.broadcast_to(b2_ref[...].astype(F32)[None, :], (128, D)).T
    c_w1.wait()
    c_w2.wait()

    def ocp(i, slot):
        return pltpu.make_async_copy(ob_v.at[slot], o_hbm.at[:, pl.ds(pl.multiple_of(i * T, T), T)], sem_o.at[slot])

    def phase2(i, c):
        st = pl.multiple_of(i * T, T)
        slot = i % 2
        xn = xn_v[:, pl.ds(st, T)]
        pq = _dot(wt_v[0:H * HP, :], xn, NN)
        qp, qn = _dual_softmax(pq, dh)
        os_ = []
        for g in range(G):
            sl = slice(g * 128, (g + 1) * 128)
            num = _dot(kvb_v[g, :, 0:128], qp[sl], NN) + _dot(kvb_v[g, :, 128:256], qn[sl], NN)
            num = num.reshape(4, HP, T)
            den = num[:, dh:dh + 1, :] + 1e-6
            os_.append((num * (1.0 / den)).reshape(128, T).astype(BF16))
        ot = jnp.concatenate(os_, axis=0)
        hid = _gelu(_dot(w1_v[...], xn, TN) + jnp.tile(b1_v[...], (1, T // 128))).astype(BF16)
        acc = _dot(w2_v[...], hid, NN) + _dot(wop_v[...], ot, NN)
        acc = acc + jnp.tile(b2_v[...], (1, T // 128)) + x_v[:, pl.ds(st, T)].astype(F32)

        @pl.when(i >= 2)
        def _():
            ocp(i - 2, slot).wait()
        ob_v[slot] = acc.astype(BF16)
        ocp(i, slot).start()
        return c

    lax.fori_loop(0, nt, phase2, 0)
    ocp(nt - 2, nt % 2).wait()
    ocp(nt - 1, (nt - 1) % 2).wait()


@jax.jit
def pallas_parallel_sum__linear_kernel_hedgehog__dense_activation_gelu__prompt_kernel(
    A_x, A_wqkv, A_w_phi, A_wo, B_x, B_w1, B_b1, B_w2, B_b2,
):
    B, S, D = A_x.shape
    FF = B_w1.shape[1]
    x = A_x.reshape(S, D).T
    any_ = pl.BlockSpec(memory_space=pltpu.HBM)
    vm = pl.BlockSpec(memory_space=pltpu.VMEM)
    out = pl.pallas_call(
        functools.partial(_kernel, S=S, D=D, FF=FF),
        in_specs=[any_, any_, vm, any_, any_, vm, any_, vm],
        out_specs=any_,
        out_shape=jax.ShapeDtypeStruct((D, S), A_x.dtype),
        scratch_shapes=[
            pltpu.VMEM((D, S), BF16), pltpu.VMEM((D, S), BF16),
            pltpu.VMEM((D, 3 * D), BF16), pltpu.VMEM((D, D), BF16),
            pltpu.VMEM((D, FF), BF16), pltpu.VMEM((D, FF), BF16),
            pltpu.VMEM((3 * D + 64, H * HP), F32), pltpu.VMEM((3 * H * HP, D), BF16),
            pltpu.VMEM((D, H * HP), BF16), pltpu.VMEM((FF, D), BF16),
            pltpu.VMEM((FF, 128), F32), pltpu.VMEM((D, 128), F32),
            pltpu.VMEM((4, 128, 256), F32), pltpu.VMEM((4, 128, 256), BF16),
            pltpu.VMEM((2, D, T), BF16),
            pltpu.SemaphoreType.DMA((S // T,)), pltpu.SemaphoreType.DMA((4,)),
            pltpu.SemaphoreType.DMA((2,)),
        ],
        compiler_params=pltpu.CompilerParams(vmem_limit_bytes=64 * 1024 * 1024),
    )(x, A_wqkv, A_w_phi.transpose(1, 0, 2), A_wo, B_w1, B_b1, B_w2.T, B_b2)
    return out.T.reshape(B, S, D)
```
